```python
import jax
import jax.numpy as jnp

def _softmax(x, axis=-1):
    return jax.nn.softmax(x, axis=axis)
def _gelu(x):
    return jax.nn.gelu(x, approximate=True)
def _silu(x):
    return jax.nn.silu(x)
def _sigmoid(x):
    return jax.nn.sigmoid(x)
def _layernorm(x, axis=-1, eps=1e-5):
    m = jnp.mean(x, axis=axis, keepdims=True)
    v = jnp.var(x, axis=axis, keepdims=True)
    return (x - m) / jnp.sqrt(v + eps)
def _scatter_add(tgt, idx, src, axis=0):
    return tgt.at[idx].add(src)
def _segment_sum(src, seg, n):
    return jax.ops.segment_sum(src, seg, n)
class _Rng:
    def __init__(self, key):
        self._k = key
    def _next(self):
        self._k, sub = jax.random.split(self._k)
        return sub
    def normal(self, shape):
        return jax.random.normal(self._next(), shape, dtype=jnp.bfloat16)
    def randint(self, lo, hi, shape):
        return jax.random.randint(self._next(), shape, lo, hi, dtype=jnp.int32)
    def uniform(self, shape, lo=0.0, hi=1.0):
        return jax.random.uniform(self._next(), shape, jnp.bfloat16, lo, hi)
    def permutation(self, n):
        return jax.random.permutation(self._next(), n)


kernel_name = 'gated_mix__sliding_local_dilated__compressed_kv_cla__prompt'

def setup_inputs():
    _rng = _Rng(jax.random.key(int.from_bytes(__import__("os").urandom(4), "little")))
    _w = (lambda a: (lambda t: t.astype(jnp.bfloat16) if jnp.issubdtype(t.dtype, jnp.floating) else t)(jnp.asarray(a)))
    def _A_setup():
        B, S, D = 1, 2048, 576
        return {
            "x": _w((lambda *s: _rng.normal(s) * 0.05)(B, S, D)),
            "wqkv": _w((lambda *s: _rng.normal(s) * 0.05)(D, 3 * D)),
            "wo": _w((lambda *s: _rng.normal(s) * 0.05)(D, D)),
        }
    _A_in = _A_setup()

    def _B_setup():
        B, H, Sq, Sk, D, M = 1, 32, 2048, 2048, 128, 576
        Dc = 4 * D
        return {
            "x": _w((lambda *s: _rng.normal(s) * 0.05)(B, Sq, M)),
            "c_kv": _w((lambda *s: _rng.normal(s) * 0.05)(B, Sk, Dc)),
            "w_q": _w((lambda *s: _rng.normal(s) * 0.05)(M, H, D) * (M ** -0.5)),
            "w_uk": _w((lambda *s: _rng.normal(s) * 0.05)(Dc, H, D) * (Dc ** -0.5)),
            "w_uv": _w((lambda *s: _rng.normal(s) * 0.05)(Dc, H, D) * (Dc ** -0.5)),
            "w_o": _w((lambda *s: _rng.normal(s) * 0.05)(H, D, M) * ((H * D) ** -0.5)),
        }
    _B_in = _B_setup()

    return {
        "A_x": _A_in["x"],
        "A_wqkv": _A_in["wqkv"],
        "A_wo": _A_in["wo"],
        "B_x": _B_in["x"],
        "B_c_kv": _B_in["c_kv"],
        "B_w_q": _B_in["w_q"],
        "B_w_uk": _B_in["w_uk"],
        "B_w_uv": _B_in["w_uv"],
        "B_w_o": _B_in["w_o"],
        "gate_w": _w((lambda *s: _rng.normal(s) * 0.05)(576)),
    }

def reference(A_x, A_wqkv, A_wo, B_x, B_c_kv, B_w_q, B_w_uk, B_w_uv, B_w_o, gate_w):
    def _A_ref(x, wqkv, wo):
        B, S, D = x.shape
        H = 32; Dh = D // H
        W, dil = 8, 2
        qkv = (lambda x, *d: x.transpose(*d))((x @ wqkv).reshape(B, S, 3, H, Dh), 2, 0, 3, 1, 4)
        q, k, v = qkv[0], qkv[1], qkv[2]
        scale = Dh ** -0.5
        pos = jnp.arange(S)
        off = jnp.arange(W) * dil
        idx = pos[:, None] - off[None, :]
        mask = idx >= 0
        idx_c = jnp.where(mask, idx, 0).reshape(-1)
        kg = k[:, :, idx_c, :].reshape(B, H, S, W, Dh)
        vg = v[:, :, idx_c, :].reshape(B, H, S, W, Dh)
        logits = jnp.einsum("bhsd,bhswd->bhsw", q, kg) * scale
        logits = jnp.where(mask[None, None, :, :], logits, -1e9)
        attn = _softmax(logits, axis=-1)
        o = jnp.einsum("bhsw,bhswd->bhsd", attn, vg)
        return (lambda x, *d: x.transpose(*d))(o, 0, 2, 1, 3).reshape(B, S, D) @ wo

    def _B_ref(x, c_kv, w_q, w_uk, w_uv, w_o):
        B, Sq, M = x.shape[0], x.shape[1], x.shape[2]
        Sk = c_kv.shape[1]
        H, D = w_q.shape[1], w_q.shape[2]
        q = jnp.einsum("bqm,mhd->bhqd", x, w_q)
        k = jnp.einsum("bkc,chd->bhkd", c_kv, w_uk)
        v = jnp.einsum("bkc,chd->bhkd", c_kv, w_uv)
        scores = jnp.einsum("bhqd,bhkd->bhqk", q, k) * (D ** -0.5)
        off = Sk - Sq
        qi = jnp.arange(Sq)[:, None]
        kj = jnp.arange(Sk)[None, :]
        cmask = kj <= (qi + off)
        scores = jnp.where(cmask[None, None], scores, -1e9)
        p = _softmax(scores, axis=-1)
        ctx = jnp.einsum("bhqk,bhkd->bhqd", p, v)
        return jnp.einsum("bhqd,hdm->bqm", ctx, w_o)

    x = A_x
    g = _sigmoid((x * gate_w).sum(-1, keepdims=True))
    a = _A_ref(x, A_wqkv, A_wo)
    b = _B_ref(x, B_c_kv, B_w_q, B_w_uk, B_w_uv, B_w_o)
    return g * a + (1 - g) * b
```

```python
import functools
import jax
import jax.numpy as jnp
import numpy as np
import jax.experimental.pallas as pl
import jax.experimental.pallas.tpu as pltpu

G = 2
BQ = 256
AH, AW, ADIL = 32, 8, 2
PADR = 16
LOG2E = 1.4426950408889634
NT = (((1,), (1,)), ((), ()))
f32, bf16 = jnp.float32, jnp.bfloat16


def _kernel(x_ref, wqkv_ref, wo_ref, c_ref, wq_ref, wk_ref, wv_ref, wout_ref, gw_ref, o_ref,
            acc_ref, q_ref, k_ref, v_ref, ctx_ref, wt_ref, wp_ref, wop_ref, ka_ref, va_ref):
    step = pl.program_id(0)
    S, M = x_ref.shape
    D = 128
    DH = M // AH
    NTILE = pl.cdiv(M, 128)
    MP = NTILE * 128
    x = x_ref[...]
    c = c_ref[...]
    q_ref[...] = (jnp.dot(x, wq_ref[...], preferred_element_type=f32) * (D ** -0.5 * LOG2E)).astype(bf16)
    k_ref[...] = jnp.dot(c, wk_ref[...], preferred_element_type=f32).astype(bf16)
    v_ref[...] = jnp.dot(c, wv_ref[...], preferred_element_type=f32).astype(bf16)
    row = jax.lax.broadcasted_iota(jnp.int32, (BQ, BQ), 0)
    col = jax.lax.broadcasted_iota(jnp.int32, (BQ, BQ), 1)
    causal = col <= row
    for g in range(G):
        hs = slice(g * D, (g + 1) * D)
        for i in range(S // BQ):
            r0, r1 = i * BQ, (i + 1) * BQ
            q = q_ref[r0:r1, hs]
            sd = jax.lax.dot_general(q, k_ref[r0:r1, hs], NT, preferred_element_type=f32)
            sd = jnp.where(causal, sd, -1e9)
            m = jnp.max(sd, axis=-1, keepdims=True)
            if i > 0:
                s = jax.lax.dot_general(q, k_ref[0:r0, hs], NT, preferred_element_type=f32)
                m = jnp.maximum(m, jnp.max(s, axis=-1, keepdims=True))
            pd = jnp.exp2(sd - m)
            l = jnp.sum(pd, axis=-1, keepdims=True)
            o = jnp.dot(pd.astype(bf16), v_ref[r0:r1, hs], preferred_element_type=f32)
            if i > 0:
                p = jnp.exp2(s - m)
                l = l + jnp.sum(p, axis=-1, keepdims=True)
                o = o + jnp.dot(p.astype(bf16), v_ref[0:r0, hs], preferred_element_type=f32)
            ctx_ref[r0:r1, hs] = (o / l).astype(bf16)
    upd = jnp.dot(ctx_ref[...], wout_ref[...], preferred_element_type=f32)

    @pl.when(step == 0)
    def _():
        acc_ref[...] = upd

    @pl.when(step > 0)
    def _():
        acc_ref[...] += upd

    @pl.when(step == pl.num_programs(0) - 1)
    def _():
        wp_ref[...] = jnp.zeros(wp_ref.shape, bf16)
        wop_ref[...] = jnp.zeros(wop_ref.shape, bf16)
        for kt in range(NTILE):
            kw = min(128, M - kt * 128)
            ks = slice(kt * 128, kt * 128 + kw)
            wt_ref[:, 0:kw] = wqkv_ref[ks, :].astype(f32).T
            for t in range(3):
                for d in range(DH):
                    wp_ref[t * MP + d * AH:t * MP + (d + 1) * AH, ks] = (
                        wt_ref[pl.ds(t * M + d, AH, stride=DH), :][:, 0:kw].astype(bf16))
            wt_ref[0:M, 0:kw] = wo_ref[:, ks].astype(f32)
            for d in range(DH):
                wop_ref[d * AH:(d + 1) * AH, ks] = wt_ref[pl.ds(d, AH, stride=DH), :][:, 0:kw].astype(bf16)
        ka_ref[:, 0:PADR, :] = jnp.zeros((NTILE, PADR, 128), f32)
        va_ref[:, 0:PADR, :] = jnp.zeros((NTILE, PADR, 128), f32)
        CH = 256

        def chunk(j, carry):
            r0 = pl.multiple_of(j * CH, CH)
            xc = x_ref[pl.ds(r0, CH), :]
            qkv = jax.lax.dot_general(xc, wp_ref[...], NT, preferred_element_type=f32)
            qkv = qkv.astype(bf16).astype(f32)
            for t in range(NTILE):
                ka_ref[t, pl.ds(r0 + PADR, CH), :] = qkv[:, MP + t * 128:MP + (t + 1) * 128]
                va_ref[t, pl.ds(r0 + PADR, CH), :] = qkv[:, 2 * MP + t * 128:2 * MP + (t + 1) * 128]
            pos = r0 + jax.lax.broadcasted_iota(jnp.int32, (CH, 128), 0)
            lg = []
            for w in range(AW):
                a = None
                for t in range(NTILE):
                    pr = qkv[:, t * 128:(t + 1) * 128] * ka_ref[t, pl.ds(r0 + (PADR - ADIL * w), CH), :]
                    a = pr if a is None else a + pr
                a = a + pltpu.roll(a, 64, 1)
                a = a + pltpu.roll(a, 32, 1)
                lg.append(jnp.where(pos >= ADIL * w, a * (DH ** -0.5), -1e9))
            mx = functools.reduce(jnp.maximum, lg)
            e = [jnp.exp(a - mx) for a in lg]
            inv = 1.0 / functools.reduce(jnp.add, e)
            outs = []
            for t in range(NTILE):
                a = None
                for w in range(AW):
                    pr = e[w] * va_ref[t, pl.ds(r0 + (PADR - ADIL * w), CH), :]
                    a = pr if a is None else a + pr
                outs.append((a * inv).astype(bf16))
            oa = jnp.dot(jnp.concatenate(outs, axis=1), wop_ref[...], preferred_element_type=f32)
            gate = jax.nn.sigmoid(jnp.sum(xc.astype(f32) * gw_ref[...].astype(f32), axis=-1, keepdims=True))
            o_ref[pl.ds(r0, CH), :] = (gate * oa + (1.0 - gate) * acc_ref[pl.ds(r0, CH), :]).astype(o_ref.dtype)
            return carry

        jax.lax.fori_loop(0, S // CH, chunk, 0)


@jax.jit
def pallas_gated_mix__sliding_local_dilated__compressed_kv_cla__prompt_kernel(
        A_x, A_wqkv, A_wo, B_x, B_c_kv, B_w_q, B_w_uk, B_w_uv, B_w_o, gate_w):
    _, S, M = A_x.shape
    _, H, D = B_w_q.shape
    C = B_c_kv.shape[-1]
    MP = pl.cdiv(M, 128) * 128
    full = lambda shape: pl.BlockSpec(shape, lambda h: (0,) * len(shape))
    out = pl.pallas_call(
        _kernel,
        grid=(H // G,),
        in_specs=[full((S, M)), full((M, 3 * M)), full((M, M)), full((S, C)),
                  pl.BlockSpec((M, G * D), lambda h: (0, h)),
                  pl.BlockSpec((C, G * D), lambda h: (0, h)),
                  pl.BlockSpec((C, G * D), lambda h: (0, h)),
                  pl.BlockSpec((G * D, M), lambda h: (h, 0)),
                  full((1, M))],
        out_specs=full((S, M)),
        out_shape=jax.ShapeDtypeStruct((S, M), A_x.dtype),
        scratch_shapes=[pltpu.VMEM((S, M), f32)] + [pltpu.VMEM((S, G * D), bf16)] * 4 + [
            pltpu.VMEM((3 * M, 128), f32), pltpu.VMEM((3 * MP, M), bf16), pltpu.VMEM((MP, M), bf16),
            pltpu.VMEM((MP // 128, S + PADR, 128), f32), pltpu.VMEM((MP // 128, S + PADR, 128), f32)],
        compiler_params=pltpu.CompilerParams(dimension_semantics=("arbitrary",),
                                             vmem_limit_bytes=100 * 1024 * 1024),
    )(A_x[0], A_wqkv, A_wo, B_c_kv[0], B_w_q.reshape(M, H * D), B_w_uk.reshape(C, H * D),
      B_w_uv.reshape(C, H * D), B_w_o.reshape(H * D, M), gate_w.reshape(1, M))
    return out[None]
```

```python
import functools
import jax
import jax.numpy as jnp
import numpy as np
import jax.experimental.pallas as pl
import jax.experimental.pallas.tpu as pltpu

G = 2
BQ = 256
D = 128
AH, AW, ADIL = 32, 8, 2
PADR = 16
LOG2E = 1.4426950408889634
NT = (((1,), (1,)), ((), ()))
f32, bf16, u32 = jnp.float32, jnp.bfloat16, jnp.uint32


def _unpack_pair(u):
    lo = pltpu.bitcast(u << 16, f32).astype(bf16)
    hi = pltpu.bitcast(u & np.uint32(0xFFFF0000), f32).astype(bf16)
    return jnp.concatenate([lo, hi], axis=1)


def _kernel(xt_ref, wqkv_ref, wo_ref, c_ref, wq_hbm, wk_hbm, wv_hbm, wout_ref, gw_ref, o_ref,
            acc_ref, ga_ref, x_ref, q_ref, k_ref, v_ref, ctx_ref, wt_ref, wp_ref, wop_ref, ka_ref, va_ref,
            wqb, wkb, wvb, sems):
    step = pl.program_id(0)
    nsteps = pl.num_programs(0)
    M, S = xt_ref.shape
    DH = M // AH
    NTILE = pl.cdiv(M, 128)
    MP = NTILE * 128

    def w_copies(p, slot):
        return [pltpu.make_async_copy(h.bitcast(u32).at[:, p, :], b.at[slot], sems.at[i, slot])
                for i, (h, b) in enumerate(((wq_hbm, wqb), (wk_hbm, wkb), (wv_hbm, wvb)))]

    @pl.when(step == 0)
    def _():
        for cp in w_copies(0, 0):
            cp.start()
        x_ref[...] = xt_ref[...].T
        wp_ref[...] = jnp.zeros(wp_ref.shape, bf16)
        for kt in range(NTILE):
            kw = min(128, M - kt * 128)
            ks = slice(kt * 128, kt * 128 + kw)
            wt_ref[:, 0:kw] = wqkv_ref[ks, :].astype(f32).T
            for t in range(3):
                for d in range(DH):
                    wp_ref[t * MP + d * AH:t * MP + (d + 1) * AH, ks] = (
                        wt_ref[pl.ds(t * M + d, AH, stride=DH), :][:, 0:kw].astype(bf16))
            wt_ref[0:M, 0:kw] = wo_ref[:, ks].astype(f32)
            wt_ref[2 * M:M + MP, :] = jnp.zeros((MP - M, 128), f32)
            for d in range(DH):
                wt_ref[M + d * AH:M + (d + 1) * AH, :] = wt_ref[pl.ds(d, AH, stride=DH), :]
            wop_ref[ks, :] = wt_ref[M:M + MP, :].T[0:kw, :].astype(bf16)
        ka_ref[:, 0:PADR, :] = jnp.zeros((NTILE, PADR, 128), f32)
        va_ref[:, 0:PADR, :] = jnp.zeros((NTILE, PADR, 128), f32)
        CH = 256

        def chunk(j, carry):
            r0 = pl.multiple_of(j * CH, CH)
            xc = x_ref[pl.ds(r0, CH), :]
            qkv = jax.lax.dot_general(xc, wp_ref[...], NT, preferred_element_type=f32)
            for t in range(NTILE):
                ka_ref[t, pl.ds(r0 + PADR, CH), :] = qkv[:, MP + t * 128:MP + (t + 1) * 128]
                va_ref[t, pl.ds(r0 + PADR, CH), :] = qkv[:, 2 * MP + t * 128:2 * MP + (t + 1) * 128]
            pos = r0 + jax.lax.broadcasted_iota(jnp.int32, (CH, 128), 0)
            lg = []
            for w in range(AW):
                a = None
                for t in range(NTILE):
                    pr = qkv[:, t * 128:(t + 1) * 128] * ka_ref[t, pl.ds(r0 + (PADR - ADIL * w), CH), :]
                    a = pr if a is None else a + pr
                a = a + pltpu.roll(a, 64, 1)
                a = a + pltpu.roll(a, 32, 1)
                lg.append(jnp.where(pos >= ADIL * w, a * (DH ** -0.5), -1e9))
            mx = functools.reduce(jnp.maximum, lg)
            e = [jnp.exp(a - mx) for a in lg]
            inv = 1.0 / functools.reduce(jnp.add, e)
            outs = []
            for t in range(NTILE):
                a = None
                for w in range(AW):
                    pr = e[w] * va_ref[t, pl.ds(r0 + (PADR - ADIL * w), CH), :]
                    a = pr if a is None else a + pr
                outs.append((a * inv).astype(bf16))
            ga_ref[:, pl.ds(r0, CH)] = jax.lax.dot_general(
                wop_ref[...], jnp.concatenate(outs, axis=1), NT, preferred_element_type=f32)
            return carry

        jax.lax.fori_loop(0, S // CH, chunk, 0)

    slot = step % 2
    for cp in w_copies(step, slot):
        cp.wait()

    @pl.when(step + 1 < nsteps)
    def _():
        for cp in w_copies(step + 1, 1 - slot):
            cp.start()

    c = c_ref[...]
    q_ref[...] = (jnp.dot(x_ref[...], _unpack_pair(wqb[slot]), preferred_element_type=f32)
                  * (D ** -0.5 * LOG2E)).astype(bf16)
    k_ref[...] = jnp.dot(c, _unpack_pair(wkb[slot]), preferred_element_type=f32).astype(bf16)
    v_ref[...] = jnp.dot(c, _unpack_pair(wvb[slot]), preferred_element_type=f32).astype(bf16)
    row = jax.lax.broadcasted_iota(jnp.int32, (BQ, BQ), 0)
    col = jax.lax.broadcasted_iota(jnp.int32, (BQ, BQ), 1)
    causal = col <= row
    for g in range(G):
        hs = slice(g * D, (g + 1) * D)
        for i in range(S // BQ):
            r0, r1 = i * BQ, (i + 1) * BQ
            q = q_ref[r0:r1, hs]
            sd = jax.lax.dot_general(q, k_ref[r0:r1, hs], NT, preferred_element_type=f32)
            sd = jnp.where(causal, sd, -1e9 * LOG2E)
            m = jnp.max(sd, axis=-1, keepdims=True)
            if i > 0:
                s = jax.lax.dot_general(q, k_ref[0:r0, hs], NT, preferred_element_type=f32)
                m = jnp.maximum(m, jnp.max(s, axis=-1, keepdims=True))
            pd = jnp.exp2(sd - m)
            l = jnp.sum(pd, axis=-1, keepdims=True)
            o = jnp.dot(pd.astype(bf16), v_ref[r0:r1, hs], preferred_element_type=f32)
            if i > 0:
                p = jnp.exp2(s - m)
                l = l + jnp.sum(p, axis=-1, keepdims=True)
                o = o + jnp.dot(p.astype(bf16), v_ref[0:r0, hs], preferred_element_type=f32)
            ctx_ref[r0:r1, hs] = (o / l).astype(bf16)
    wo_t = jnp.concatenate([wout_ref[g] for g in range(G)], axis=1)
    upd = jax.lax.dot_general(wo_t, ctx_ref[...], NT, preferred_element_type=f32)

    @pl.when(step == 0)
    def _():
        acc_ref[...] = upd

    @pl.when(step > 0)
    def _():
        acc_ref[...] += upd

    @pl.when(step == nsteps - 1)
    def _():
        gw = jnp.broadcast_to(gw_ref[...], (16, M))
        gate = jax.nn.sigmoid(jnp.dot(gw, xt_ref[...], preferred_element_type=f32)[0:1, :])
        o_ref[...] = (gate * ga_ref[...] + (1.0 - gate) * acc_ref[...]).astype(o_ref.dtype)


@jax.jit
def pallas_gated_mix__sliding_local_dilated__compressed_kv_cla__prompt_kernel(
        A_x, A_wqkv, A_wo, B_x, B_c_kv, B_w_q, B_w_uk, B_w_uv, B_w_o, gate_w):
    _, S, M = A_x.shape
    _, H, _ = B_w_q.shape
    C = B_c_kv.shape[-1]
    MP = pl.cdiv(M, 128) * 128
    full = lambda shape: pl.BlockSpec(shape, lambda h: (0,) * len(shape))
    hbm = pl.BlockSpec(memory_space=pl.ANY)
    out = pl.pallas_call(
        _kernel,
        grid=(H // G,),
        in_specs=[full((M, S)), full((M, 3 * M)), full((M, M)), full((S, C)), hbm, hbm, hbm,
                  pl.BlockSpec((G, M, D), lambda h: (h, 0, 0)),
                  full((1, M))],
        out_specs=full((M, S)),
        out_shape=jax.ShapeDtypeStruct((M, S), A_x.dtype),
        scratch_shapes=[pltpu.VMEM((M, S), f32), pltpu.VMEM((M, S), f32), pltpu.VMEM((S, M), bf16)]
        + [pltpu.VMEM((S, G * D), bf16)] * 4 + [
            pltpu.VMEM((3 * M, 128), f32), pltpu.VMEM((3 * MP, M), bf16), pltpu.VMEM((M, MP), bf16),
            pltpu.VMEM((MP // 128, S + PADR, 128), f32), pltpu.VMEM((MP // 128, S + PADR, 128), f32),
            pltpu.VMEM((2, M, D), u32), pltpu.VMEM((2, C, D), u32), pltpu.VMEM((2, C, D), u32),
            pltpu.SemaphoreType.DMA((3, 2))],
        compiler_params=pltpu.CompilerParams(dimension_semantics=("arbitrary",),
                                             vmem_limit_bytes=100 * 1024 * 1024),
    )(A_x[0].T, A_wqkv, A_wo, B_c_kv[0], B_w_q, B_w_uk, B_w_uv, B_w_o.transpose(0, 2, 1), gate_w.reshape(1, M))
    return out.T[None]
```

```python
import functools
import jax
import jax.numpy as jnp
import numpy as np
import jax.experimental.pallas as pl
import jax.experimental.pallas.tpu as pltpu

G = 2
BQ = 256
D = 128
AH, AW, ADIL = 32, 8, 2
PADR = 16
LOG2E = 1.4426950408889634
NT = (((1,), (1,)), ((), ()))
f32, bf16, u32 = jnp.float32, jnp.bfloat16, jnp.uint32


def _unpack_pair(u):
    lo = pltpu.bitcast(u << 16, f32).astype(bf16)
    hi = pltpu.bitcast(u & np.uint32(0xFFFF0000), f32).astype(bf16)
    return jnp.concatenate([lo, hi], axis=1)


def _kernel(xt_ref, wqkv_ref, wo_ref, c_ref, wq_hbm, wk_hbm, wv_hbm, wout_ref, gw_ref, o_ref,
            acc_ref, oa_ref, qa_ref, x_ref, q_ref, k_ref, v_ref, ctx_ref, wt_ref, wp_ref, wop_ref, ka_ref, va_ref,
            wqb, wkb, wvb, sems):
    step = pl.program_id(0)
    nsteps = pl.num_programs(0)
    M, S = xt_ref.shape
    DH = M // AH
    NTILE = pl.cdiv(M, 128)
    MP = NTILE * 128

    def w_copies(p, slot):
        return [pltpu.make_async_copy(h.bitcast(u32).at[:, p, :], b.at[slot], sems.at[i, slot])
                for i, (h, b) in enumerate(((wq_hbm, wqb), (wk_hbm, wkb), (wv_hbm, wvb)))]

    @pl.when(step == 0)
    def _():
        for cp in w_copies(0, 0):
            cp.start()
        x_ref[...] = xt_ref[...].T
        wp_ref[...] = jnp.zeros(wp_ref.shape, bf16)
        for kt in range(NTILE):
            kw = min(128, M - kt * 128)
            ks = slice(kt * 128, kt * 128 + kw)
            wt_ref[:, 0:kw] = wqkv_ref[ks, :].astype(f32).T
            for t in range(3):
                for d in range(DH):
                    wp_ref[t * MP + d * AH:t * MP + (d + 1) * AH, ks] = (
                        wt_ref[pl.ds(t * M + d, AH, stride=DH), :][:, 0:kw].astype(bf16))
            wt_ref[0:M, 0:kw] = wo_ref[:, ks].astype(f32)
            wt_ref[2 * M:M + MP, :] = jnp.zeros((MP - M, 128), f32)
            for d in range(DH):
                wt_ref[M + d * AH:M + (d + 1) * AH, :] = wt_ref[pl.ds(d, AH, stride=DH), :]
            wop_ref[ks, :] = wt_ref[M:M + MP, :].T[0:kw, :].astype(bf16)
        ka_ref[:, 0:PADR, :] = jnp.zeros((NTILE, PADR, 128), f32)
        va_ref[:, 0:PADR, :] = jnp.zeros((NTILE, PADR, 128), f32)
        acc_ref[...] = jnp.zeros(acc_ref.shape, f32)
        CH = 512

        def chunk(j, carry):
            r0 = pl.multiple_of(j * CH, CH)
            qkv = jax.lax.dot_general(x_ref[pl.ds(r0, CH), :], wp_ref[...], NT, preferred_element_type=f32)
            for t in range(NTILE):
                qa_ref[t, pl.ds(r0, CH), :] = qkv[:, t * 128:(t + 1) * 128] * (DH ** -0.5)
                ka_ref[t, pl.ds(r0 + PADR, CH), :] = qkv[:, MP + t * 128:MP + (t + 1) * 128]
                va_ref[t, pl.ds(r0 + PADR, CH), :] = qkv[:, 2 * MP + t * 128:2 * MP + (t + 1) * 128]
            return carry

        jax.lax.fori_loop(0, S // CH, chunk, 0)

    def local_attn(r0, n):
        pos = r0 + jax.lax.broadcasted_iota(jnp.int32, (n, 128), 0)
        qa = [qa_ref[t, pl.ds(r0, n), :] for t in range(NTILE)]
        lg = []
        for w in range(AW):
            a = None
            for t in range(NTILE):
                pr = qa[t] * ka_ref[t, pl.ds(r0 + (PADR - ADIL * w), n), :]
                a = pr if a is None else a + pr
            a = a + pltpu.roll(a, 64, 1)
            a = a + pltpu.roll(a, 32, 1)
            lg.append(jnp.where(pos >= ADIL * w, a, -1e9))
        mx = functools.reduce(jnp.maximum, lg)
        e = [jnp.exp(a - mx) for a in lg]
        inv = 1.0 / functools.reduce(jnp.add, e)
        for t in range(NTILE):
            a = None
            for w in range(AW):
                pr = e[w] * va_ref[t, pl.ds(r0 + (PADR - ADIL * w), n), :]
                a = pr if a is None else a + pr
            oa_ref[pl.ds(r0, n), t * 128:(t + 1) * 128] = (a * inv).astype(bf16)

    slot = step % 2
    for cp in w_copies(step, slot):
        cp.wait()

    @pl.when(step + 1 < nsteps)
    def _():
        for cp in w_copies(step + 1, 1 - slot):
            cp.start()

    c = c_ref[...]
    q_ref[...] = (jnp.dot(x_ref[...], _unpack_pair(wqb[slot]), preferred_element_type=f32)
                  * (D ** -0.5 * LOG2E)).astype(bf16)
    k_ref[...] = jnp.dot(c, _unpack_pair(wkb[slot]), preferred_element_type=f32).astype(bf16)
    v_ref[...] = jnp.dot(c, _unpack_pair(wvb[slot]), preferred_element_type=f32).astype(bf16)
    HB = BQ // 2
    causal = (jax.lax.broadcasted_iota(jnp.int32, (HB, HB), 1)
              <= jax.lax.broadcasted_iota(jnp.int32, (HB, HB), 0))
    NEG = -1e9 * LOG2E
    nblk = S // BQ
    arows = S // nsteps // nblk
    for g in range(G):
        hs = slice(g * D, (g + 1) * D)
        for i in range(nblk):
            if (g * nblk + i) % G == 0:
                local_attn(pl.multiple_of(step * (S // nsteps) + (g * nblk + i) // G * arows, arows), arows)
            r0, rm, r1 = i * BQ, i * BQ + HB, (i + 1) * BQ
            q = q_ref[r0:r1, hs]
            s = jax.lax.dot_general(q, k_ref[0:rm, hs], NT, preferred_element_type=f32)
            sd = jax.lax.dot_general(q[HB:], k_ref[rm:r1, hs], NT, preferred_element_type=f32)
            sd = jnp.where(causal, sd, NEG)
            st = jnp.where(causal, s[:HB, r0:], NEG)
            if i > 0:
                st = jnp.concatenate([s[:HB, :r0], st], axis=1)
            sb = s[HB:]
            pt = jnp.exp2(st - jnp.max(st, axis=-1, keepdims=True))
            mb = jnp.maximum(jnp.max(sb, axis=-1, keepdims=True), jnp.max(sd, axis=-1, keepdims=True))
            pb = jnp.exp2(sb - mb)
            pd = jnp.exp2(sd - mb)
            lt = jnp.sum(pt, axis=-1, keepdims=True)
            lb = jnp.sum(pb, axis=-1, keepdims=True) + jnp.sum(pd, axis=-1, keepdims=True)
            o = jnp.dot(jnp.concatenate([pt, pb], axis=0).astype(bf16), v_ref[0:rm, hs],
                        preferred_element_type=f32)
            od = jnp.dot(pd.astype(bf16), v_ref[rm:r1, hs], preferred_element_type=f32)
            ctx_ref[r0:rm, hs] = (o[:HB] / lt).astype(bf16)
            ctx_ref[rm:r1, hs] = ((o[HB:] + od) / lb).astype(bf16)
    wo_t = jnp.concatenate([wout_ref[g] for g in range(G)], axis=1)
    acc_ref[...] += jax.lax.dot_general(wo_t, ctx_ref[...], NT, preferred_element_type=f32)

    @pl.when(step == nsteps - 1)
    def _():
        gate = jax.nn.sigmoid(jnp.sum(x_ref[...].astype(f32) * gw_ref[...].astype(f32), axis=-1, keepdims=True))
        gate = jnp.broadcast_to(gate, (S, 128)).T[0:1, :]
        oa = jax.lax.dot_general(wop_ref[...], oa_ref[...], NT, preferred_element_type=f32)
        o_ref[...] = (gate * oa + (1.0 - gate) * acc_ref[...]).astype(o_ref.dtype)


@jax.jit
def pallas_gated_mix__sliding_local_dilated__compressed_kv_cla__prompt_kernel(
        A_x, A_wqkv, A_wo, B_x, B_c_kv, B_w_q, B_w_uk, B_w_uv, B_w_o, gate_w):
    _, S, M = A_x.shape
    _, H, _ = B_w_q.shape
    C = B_c_kv.shape[-1]
    MP = pl.cdiv(M, 128) * 128
    full = lambda shape: pl.BlockSpec(shape, lambda h: (0,) * len(shape))
    hbm = pl.BlockSpec(memory_space=pl.ANY)
    out = pl.pallas_call(
        _kernel,
        grid=(H // G,),
        in_specs=[full((M, S)), full((M, 3 * M)), full((M, M)), full((S, C)), hbm, hbm, hbm,
                  pl.BlockSpec((G, M, D), lambda h: (h, 0, 0)),
                  full((1, M))],
        out_specs=full((M, S)),
        out_shape=jax.ShapeDtypeStruct((M, S), A_x.dtype),
        scratch_shapes=[pltpu.VMEM((M, S), f32), pltpu.VMEM((S, MP), bf16), pltpu.VMEM((MP // 128, S, 128), f32),
                         pltpu.VMEM((S, M), bf16)]
        + [pltpu.VMEM((S, G * D), bf16)] * 4 + [
            pltpu.VMEM((3 * M, 128), f32), pltpu.VMEM((3 * MP, M), bf16), pltpu.VMEM((M, MP), bf16),
            pltpu.VMEM((MP // 128, S + PADR, 128), f32), pltpu.VMEM((MP // 128, S + PADR, 128), f32),
            pltpu.VMEM((2, M, D), u32), pltpu.VMEM((2, C, D), u32), pltpu.VMEM((2, C, D), u32),
            pltpu.SemaphoreType.DMA((3, 2))],
        compiler_params=pltpu.CompilerParams(dimension_semantics=("arbitrary",),
                                             vmem_limit_bytes=100 * 1024 * 1024),
    )(A_x[0].T, A_wqkv, A_wo, B_c_kv[0], B_w_q, B_w_uk, B_w_uv, B_w_o.transpose(0, 2, 1), gate_w.reshape(1, M))
    return out.T[None]
```

```python
import functools
import jax
import jax.numpy as jnp
import numpy as np
import jax.experimental.pallas as pl
import jax.experimental.pallas.tpu as pltpu

G = 2
BQ = 256
D = 128
AH, AW, ADIL = 32, 8, 2
PADR = 16
LOG2E = 1.4426950408889634
NT = (((1,), (1,)), ((), ()))
f32, bf16, u32 = jnp.float32, jnp.bfloat16, jnp.uint32


def _unpack_pair(u):
    lo = pltpu.bitcast(u << 16, f32).astype(bf16)
    hi = pltpu.bitcast(u & np.uint32(0xFFFF0000), f32).astype(bf16)
    return jnp.concatenate([lo, hi], axis=1)


def _kernel(xt_ref, wqkv_hbm, wo_hbm, c_hbm, wq_hbm, wk_hbm, wv_hbm, wout_ref, gw_ref, o_ref,
            acc_ref, oa_ref, qa_ref, x_ref, q_ref, k_ref, g_ref, ctx_ref, wt_ref, wp_ref, wop_ref, ka_ref, va_ref,
            wqb, wkb, wvb, sems, wqkv_ref, wo_ref, c_ref, sem0):
    step = pl.program_id(0)
    nsteps = pl.num_programs(0)
    M, S = xt_ref.shape
    DH = M // AH
    NTILE = pl.cdiv(M, 128)
    MP = NTILE * 128

    def w_copies(p, slot):
        return [pltpu.make_async_copy(h.bitcast(u32).at[:, p, :], b.at[slot], sems.at[i, slot])
                for i, (h, b) in enumerate(((wq_hbm, wqb), (wk_hbm, wkb), (wv_hbm, wvb)))]

    @pl.when(step == 0)
    def _():
        first = [pltpu.make_async_copy(a, b, sem0.at[i])
                 for i, (a, b) in enumerate(((wqkv_hbm, wqkv_ref), (wo_hbm, wo_ref), (c_hbm, c_ref)))]
        for cp in first + w_copies(0, 0):
            cp.start()
        x_ref[...] = xt_ref[...].T
        first[0].wait()
        first[1].wait()
        for t in range(3):
            wp_ref[t * MP + M:(t + 1) * MP, :] = jnp.zeros((MP - M, M), bf16)
        wp_ref[M:M + 16, :] = jnp.broadcast_to(gw_ref[...], (16, M))
        for kt in range(NTILE):
            kw = min(128, M - kt * 128)
            ks = slice(kt * 128, kt * 128 + kw)
            wt_ref[:, 0:kw] = wqkv_ref[ks, :].astype(f32).T
            for t in range(3):
                for d in range(DH):
                    wp_ref[t * MP + d * AH:t * MP + (d + 1) * AH, ks] = (
                        wt_ref[pl.ds(t * M + d, AH, stride=DH), :][:, 0:kw].astype(bf16))
            wt_ref[0:M, 0:kw] = wo_ref[:, ks].astype(f32)
            wt_ref[2 * M:M + MP, :] = jnp.zeros((MP - M, 128), f32)
            for d in range(DH):
                wt_ref[M + d * AH:M + (d + 1) * AH, :] = wt_ref[pl.ds(d, AH, stride=DH), :]
            wop_ref[ks, :] = wt_ref[M:M + MP, :].T[0:kw, :].astype(bf16)
        ka_ref[:, 0:PADR, :] = jnp.zeros((NTILE, PADR, 128), f32)
        va_ref[:, 0:PADR, :] = jnp.zeros((NTILE, PADR, 128), f32)
        CH = 512

        def chunk(j, carry):
            r0 = pl.multiple_of(j * CH, CH)
            qkv = jax.lax.dot_general(x_ref[pl.ds(r0, CH), :], wp_ref[...], NT, preferred_element_type=f32)
            for t in range(NTILE):
                qa_ref[t, pl.ds(r0, CH), :] = qkv[:, t * 128:(t + 1) * 128] * (DH ** -0.5)
                ka_ref[t, pl.ds(r0 + PADR, CH), :] = qkv[:, MP + t * 128:MP + (t + 1) * 128]
                va_ref[t, pl.ds(r0 + PADR, CH), :] = qkv[:, 2 * MP + t * 128:2 * MP + (t + 1) * 128]
            g_ref[pl.ds(r0, CH), :] = jax.nn.sigmoid(jnp.broadcast_to(qkv[:, M:M + 1], (CH, 128)))
            acc_ref[:, pl.ds(r0, CH)] = jnp.zeros((M, CH), f32)
            return carry

        jax.lax.fori_loop(0, S // CH, chunk, 0)
        first[2].wait()

    def local_attn(r0, n):
        pos = r0 + jax.lax.broadcasted_iota(jnp.int32, (n, 128), 0)
        qa = [qa_ref[t, pl.ds(r0, n), :] for t in range(NTILE)]
        lg = []
        for w in range(AW):
            a = None
            for t in range(NTILE):
                pr = qa[t] * ka_ref[t, pl.ds(r0 + (PADR - ADIL * w), n), :]
                a = pr if a is None else a + pr
            a = a + pltpu.roll(a, 64, 1)
            a = a + pltpu.roll(a, 32, 1)
            lg.append(jnp.where(pos >= ADIL * w, a, -1e9))
        mx = functools.reduce(jnp.maximum, lg)
        e = [jnp.exp(a - mx) for a in lg]
        inv = g_ref[pl.ds(r0, n), :] / functools.reduce(jnp.add, e)
        for t in range(NTILE):
            a = None
            for w in range(AW):
                pr = e[w] * va_ref[t, pl.ds(r0 + (PADR - ADIL * w), n), :]
                a = pr if a is None else a + pr
            oa_ref[pl.ds(r0, n), t * 128:(t + 1) * 128] = (a * inv).astype(bf16)

    slot = step % 2
    for cp in w_copies(step, slot):
        cp.wait()

    @pl.when(step + 1 < nsteps)
    def _():
        for cp in w_copies(step + 1, 1 - slot):
            cp.start()

    c = c_ref[...]
    for j in range(8):
        local_attn(pl.multiple_of(step * 128 + j * 16, 16), 16)
    q_ref[...] = (jnp.dot(x_ref[...], _unpack_pair(wqb[slot]), preferred_element_type=f32)
                  * (D ** -0.5 * LOG2E)).astype(bf16)
    k_ref[...] = jnp.dot(c, _unpack_pair(wkb[slot]), preferred_element_type=f32).astype(bf16)
    oa_ref[:, MP:] = jnp.dot(c, _unpack_pair(wvb[slot]), preferred_element_type=f32).astype(bf16)
    HB = BQ // 2
    causal = (jax.lax.broadcasted_iota(jnp.int32, (HB, HB), 1)
              <= jax.lax.broadcasted_iota(jnp.int32, (HB, HB), 0))
    NEG = -1e9 * LOG2E
    nblk = S // BQ
    arows = S // nsteps // nblk
    for g in range(G):
        hs = slice(g * D, (g + 1) * D)
        vs = slice(MP + g * D, MP + (g + 1) * D)
        for i in range(nblk):
            r0, rm, r1 = i * BQ, i * BQ + HB, (i + 1) * BQ
            q = q_ref[r0:r1, hs]
            s = jax.lax.dot_general(q, k_ref[0:rm, hs], NT, preferred_element_type=f32)
            sd = jax.lax.dot_general(q[HB:], k_ref[rm:r1, hs], NT, preferred_element_type=f32)
            sd = jnp.where(causal, sd, NEG)
            st = jnp.where(causal, s[:HB, r0:], NEG)
            if i > 0:
                st = jnp.concatenate([s[:HB, :r0], st], axis=1)
            sb = s[HB:]
            pt = jnp.exp2(st - jnp.max(st, axis=-1, keepdims=True))
            mb = jnp.maximum(jnp.max(sb, axis=-1, keepdims=True), jnp.max(sd, axis=-1, keepdims=True))
            pb = jnp.exp2(sb - mb)
            pd = jnp.exp2(sd - mb)
            lt = jnp.sum(pt, axis=-1, keepdims=True)
            lb = jnp.sum(pb, axis=-1, keepdims=True) + jnp.sum(pd, axis=-1, keepdims=True)
            o = jnp.dot(jnp.concatenate([pt, pb], axis=0).astype(bf16), oa_ref[0:rm, vs],
                        preferred_element_type=f32)
            od = jnp.dot(pd.astype(bf16), oa_ref[rm:r1, vs], preferred_element_type=f32)
            ctx_ref[r0:rm, hs] = (o[:HB] * ((1.0 - g_ref[r0:rm, :]) / lt)).astype(bf16)
            ctx_ref[rm:r1, hs] = ((o[HB:] + od) * ((1.0 - g_ref[rm:r1, :]) / lb)).astype(bf16)
    wo_t = jnp.concatenate([wout_ref[g] for g in range(G)], axis=1)
    acc_ref[...] += jax.lax.dot_general(wo_t, ctx_ref[...], NT, preferred_element_type=f32)

    @pl.when(step == nsteps - 1)
    def _():
        oa = jax.lax.dot_general(wop_ref[...], oa_ref[:, :MP], NT, preferred_element_type=f32)
        o_ref[...] = (oa + acc_ref[...]).astype(o_ref.dtype)


@jax.jit
def pallas_gated_mix__sliding_local_dilated__compressed_kv_cla__prompt_kernel(
        A_x, A_wqkv, A_wo, B_x, B_c_kv, B_w_q, B_w_uk, B_w_uv, B_w_o, gate_w):
    _, S, M = A_x.shape
    _, H, _ = B_w_q.shape
    C = B_c_kv.shape[-1]
    MP = pl.cdiv(M, 128) * 128
    full = lambda shape: pl.BlockSpec(shape, lambda h: (0,) * len(shape))
    hbm = pl.BlockSpec(memory_space=pl.ANY)
    out = pl.pallas_call(
        _kernel,
        grid=(H // G,),
        in_specs=[full((M, S)), hbm, hbm, hbm, hbm, hbm, hbm,
                  pl.BlockSpec((G, M, D), lambda h: (h, 0, 0)),
                  full((1, M))],
        out_specs=full((M, S)),
        out_shape=jax.ShapeDtypeStruct((M, S), A_x.dtype),
        scratch_shapes=[pltpu.VMEM((M, S), f32), pltpu.VMEM((S, MP + G * D), bf16), pltpu.VMEM((MP // 128, S, 128), f32),
                         pltpu.VMEM((S, M), bf16)]
        + [pltpu.VMEM((S, G * D), bf16)] * 2 + [
            pltpu.VMEM((S, 128), f32), pltpu.VMEM((S, G * D), bf16),
            pltpu.VMEM((3 * M, 128), f32), pltpu.VMEM((3 * MP, M), bf16), pltpu.VMEM((M, MP), bf16),
            pltpu.VMEM((MP // 128, S + PADR, 128), f32), pltpu.VMEM((MP // 128, S + PADR, 128), f32),
            pltpu.VMEM((2, M, D), u32), pltpu.VMEM((2, C, D), u32), pltpu.VMEM((2, C, D), u32),
            pltpu.SemaphoreType.DMA((3, 2)),
            pltpu.VMEM((M, 3 * M), bf16), pltpu.VMEM((M, M), bf16), pltpu.VMEM((S, C), bf16),
            pltpu.SemaphoreType.DMA((3,))],
        compiler_params=pltpu.CompilerParams(dimension_semantics=("arbitrary",),
                                             vmem_limit_bytes=100 * 1024 * 1024),
    )(A_x[0].T, A_wqkv, A_wo, B_c_kv[0], B_w_q, B_w_uk, B_w_uv, B_w_o.transpose(0, 2, 1), gate_w.reshape(1, M))
    return out.T[None]
```

```python
import functools
import jax
import jax.numpy as jnp
import numpy as np
import jax.experimental.pallas as pl
import jax.experimental.pallas.tpu as pltpu

G = 2
BQ = 256
D = 128
ORDER, LOOK, DELAY = (0,2,4,6,7,5,3,1), 2, 3
AH, AW, ADIL = 32, 8, 2
PADR = 16
LOG2E = 1.4426950408889634
NT = (((1,), (1,)), ((), ()))
f32, bf16, u32 = jnp.float32, jnp.bfloat16, jnp.uint32


def _unpack_pair(u):
    lo = pltpu.bitcast(u << 16, f32).astype(bf16)
    hi = pltpu.bitcast(u & np.uint32(0xFFFF0000), f32).astype(bf16)
    return jnp.concatenate([lo, hi], axis=1)


def _kernel(xt_ref, wqkv_hbm, wo_hbm, c_hbm, wq_hbm, wk_hbm, wv_hbm, wout_ref, gw_ref, o_ref,
            acc_ref, oa_ref, qa_ref, x_ref, q_ref, k_ref, g_ref, ctx_ref, wt_ref, wp_ref, wop_ref, ka_ref, va_ref,
            wqb, wkb, wvb, sems, wqkv_ref, wo_ref, c_ref, sem0):
    step = pl.program_id(0)
    nsteps = pl.num_programs(0)
    M, S = xt_ref.shape
    DH = M // AH
    NTILE = pl.cdiv(M, 128)
    MP = NTILE * 128

    def w_copies(p, slot):
        return [pltpu.make_async_copy(h.bitcast(u32).at[:, p, :], b.at[slot], sems.at[i, slot])
                for i, (h, b) in enumerate(((wq_hbm, wqb), (wk_hbm, wkb), (wv_hbm, wvb)))]

    @pl.when(step == 0)
    def _():
        first = [pltpu.make_async_copy(a, b, sem0.at[i])
                 for i, (a, b) in enumerate(((wqkv_hbm, wqkv_ref), (wo_hbm, wo_ref), (c_hbm, c_ref)))]
        for cp in first + w_copies(0, 0):
            cp.start()
        x_ref[...] = xt_ref[...].T
        first[0].wait()
        first[1].wait()
        for t in range(3):
            wp_ref[t * MP + M:(t + 1) * MP, :] = jnp.zeros((MP - M, M), bf16)
        wp_ref[M:M + 16, :] = jnp.broadcast_to(gw_ref[...], (16, M))
        for kt in range(NTILE):
            kw = min(128, M - kt * 128)
            ks = slice(kt * 128, kt * 128 + kw)
            wt_ref[:, 0:kw] = wqkv_ref[ks, :].astype(f32).T
            for t in range(3):
                for d in range(DH):
                    wp_ref[t * MP + d * AH:t * MP + (d + 1) * AH, ks] = (
                        wt_ref[pl.ds(t * M + d, AH, stride=DH), :][:, 0:kw].astype(bf16))
            wt_ref[0:M, 0:kw] = wo_ref[:, ks].astype(f32)
            wt_ref[2 * M:M + MP, :] = jnp.zeros((MP - M, 128), f32)
            for d in range(DH):
                wt_ref[M + d * AH:M + (d + 1) * AH, :] = wt_ref[pl.ds(d, AH, stride=DH), :]
            wop_ref[ks, :] = wt_ref[M:M + MP, :].T[0:kw, :].astype(bf16)
        ka_ref[:, 0:PADR, :] = jnp.zeros((NTILE, PADR, 128), f32)
        va_ref[:, 0:PADR, :] = jnp.zeros((NTILE, PADR, 128), f32)
        CH = 512

        def chunk(j, carry):
            r0 = pl.multiple_of(j * CH, CH)
            qkv = jax.lax.dot_general(x_ref[pl.ds(r0, CH), :], wp_ref[...], NT, preferred_element_type=f32)
            for t in range(NTILE):
                qa_ref[t, pl.ds(r0, CH), :] = qkv[:, t * 128:(t + 1) * 128] * (DH ** -0.5)
                ka_ref[t, pl.ds(r0 + PADR, CH), :] = qkv[:, MP + t * 128:MP + (t + 1) * 128]
                va_ref[t, pl.ds(r0 + PADR, CH), :] = qkv[:, 2 * MP + t * 128:2 * MP + (t + 1) * 128]
            g_ref[pl.ds(r0, CH), :] = jax.nn.sigmoid(jnp.broadcast_to(qkv[:, M:M + 1], (CH, 128)))
            acc_ref[:, pl.ds(r0, CH)] = jnp.zeros((M, CH), f32)
            return carry

        jax.lax.fori_loop(0, S // CH, chunk, 0)
        first[2].wait()

    def local_attn(r0, n):
        pos = r0 + jax.lax.broadcasted_iota(jnp.int32, (n, 128), 0)
        qa = [qa_ref[t, pl.ds(r0, n), :] for t in range(NTILE)]
        lg = []
        for w in range(AW):
            a = None
            for t in range(NTILE):
                pr = qa[t] * ka_ref[t, pl.ds(r0 + (PADR - ADIL * w), n), :]
                a = pr if a is None else a + pr
            a = a + pltpu.roll(a, 64, 1)
            a = a + pltpu.roll(a, 32, 1)
            lg.append(jnp.where(pos >= ADIL * w, a, -1e9))
        mx = functools.reduce(jnp.maximum, lg)
        e = [jnp.exp(a - mx) for a in lg]
        inv = g_ref[pl.ds(r0, n), :] / functools.reduce(jnp.add, e)
        for t in range(NTILE):
            a = None
            for w in range(AW):
                pr = e[w] * va_ref[t, pl.ds(r0 + (PADR - ADIL * w), n), :]
                a = pr if a is None else a + pr
            oa_ref[pl.ds(r0, n), t * 128:(t + 1) * 128] = (a * inv).astype(bf16)

    slot = step % 2
    for cp in w_copies(step, slot):
        cp.wait()

    @pl.when(step + 1 < nsteps)
    def _():
        for cp in w_copies(step + 1, 1 - slot):
            cp.start()

    c = c_ref[...]
    for j in range(8):
        local_attn(pl.multiple_of(step * 128 + j * 16, 16), 16)
    q_ref[...] = (jnp.dot(x_ref[...], _unpack_pair(wqb[slot]), preferred_element_type=f32)
                  * (D ** -0.5 * LOG2E)).astype(bf16)
    k_ref[...] = jnp.dot(c, _unpack_pair(wkb[slot]), preferred_element_type=f32).astype(bf16)
    oa_ref[:, MP:] = jnp.dot(c, _unpack_pair(wvb[slot]), preferred_element_type=f32).astype(bf16)
    HB = BQ // 2
    causal = (jax.lax.broadcasted_iota(jnp.int32, (HB, HB), 1)
              <= jax.lax.broadcasted_iota(jnp.int32, (HB, HB), 0))
    NEG = -1e9 * LOG2E
    nblk = S // BQ
    arows = S // nsteps // nblk
    wo_t = jnp.concatenate([wout_ref[g] for g in range(G)], axis=1)

    def scores(i, g):
        r0, rm, r1 = i * BQ, i * BQ + HB, (i + 1) * BQ
        hs = slice(g * D, (g + 1) * D)
        q = q_ref[r0:r1, hs]
        s = jax.lax.dot_general(q, k_ref[0:rm, hs], NT, preferred_element_type=f32)
        sd = jax.lax.dot_general(q[HB:], k_ref[rm:r1, hs], NT, preferred_element_type=f32)
        st = jnp.where(causal, s[:HB, r0:], NEG)
        if i > 0:
            st = jnp.concatenate([s[:HB, :r0], st], axis=1)
        return st, jnp.concatenate([s[HB:], jnp.where(causal, sd, NEG)], axis=1)

    def attend(i, g, st, sb):
        r0, rm, r1 = i * BQ, i * BQ + HB, (i + 1) * BQ
        hs = slice(g * D, (g + 1) * D)
        vs = slice(MP + g * D, MP + (g + 1) * D)
        pt = jnp.exp2(st - jnp.max(st, axis=-1, keepdims=True))
        pb = jnp.exp2(sb - jnp.max(sb, axis=-1, keepdims=True))
        rt = (1.0 - g_ref[r0:rm, :]) / jnp.sum(pt, axis=-1, keepdims=True)
        rb = (1.0 - g_ref[rm:r1, :]) / jnp.sum(pb, axis=-1, keepdims=True)
        pb = pb.astype(bf16)
        o = jnp.dot(jnp.concatenate([pt.astype(bf16), pb[:, :rm]], axis=0), oa_ref[0:rm, vs],
                    preferred_element_type=f32)
        od = jnp.dot(pb[:, rm:], oa_ref[rm:r1, vs], preferred_element_type=f32)
        ctx_ref[r0:rm, hs] = (o[:HB] * rt).astype(bf16)
        ctx_ref[rm:r1, hs] = ((o[HB:] + od) * rb).astype(bf16)

    def project(i):
        rs = slice(i * BQ, (i + 1) * BQ)
        acc_ref[:, rs] += jax.lax.dot_general(wo_t, ctx_ref[rs, :], NT, preferred_element_type=f32)

    units = [(i, g) for i in ORDER for g in range(G)]
    pend = [scores(*u) for u in units[:LOOK]]
    for n, u in enumerate(units):
        if n + LOOK < len(units):
            pend.append(scores(*units[n + LOOK]))
        attend(*u, *pend.pop(0))
        if n >= DELAY and units[n - DELAY][1] == G - 1:
            project(units[n - DELAY][0])
    for u in units[len(units) - DELAY:]:
        if u[1] == G - 1:
            project(u[0])

    @pl.when(step == nsteps - 1)
    def _():
        oa = jax.lax.dot_general(wop_ref[...], oa_ref[:, :MP], NT, preferred_element_type=f32)
        o_ref[...] = (oa + acc_ref[...]).astype(o_ref.dtype)


@jax.jit
def pallas_gated_mix__sliding_local_dilated__compressed_kv_cla__prompt_kernel(
        A_x, A_wqkv, A_wo, B_x, B_c_kv, B_w_q, B_w_uk, B_w_uv, B_w_o, gate_w):
    _, S, M = A_x.shape
    _, H, _ = B_w_q.shape
    C = B_c_kv.shape[-1]
    MP = pl.cdiv(M, 128) * 128
    full = lambda shape: pl.BlockSpec(shape, lambda h: (0,) * len(shape))
    hbm = pl.BlockSpec(memory_space=pl.ANY)
    out = pl.pallas_call(
        _kernel,
        grid=(H // G,),
        in_specs=[full((M, S)), hbm, hbm, hbm, hbm, hbm, hbm,
                  pl.BlockSpec((G, M, D), lambda h: (h, 0, 0)),
                  full((1, M))],
        out_specs=full((M, S)),
        out_shape=jax.ShapeDtypeStruct((M, S), A_x.dtype),
        scratch_shapes=[pltpu.VMEM((M, S), f32), pltpu.VMEM((S, MP + G * D), bf16), pltpu.VMEM((MP // 128, S, 128), f32),
                         pltpu.VMEM((S, M), bf16)]
        + [pltpu.VMEM((S, G * D), bf16)] * 2 + [
            pltpu.VMEM((S, 128), f32), pltpu.VMEM((S, G * D), bf16),
            pltpu.VMEM((3 * M, 128), f32), pltpu.VMEM((3 * MP, M), bf16), pltpu.VMEM((M, MP), bf16),
            pltpu.VMEM((MP // 128, S + PADR, 128), f32), pltpu.VMEM((MP // 128, S + PADR, 128), f32),
            pltpu.VMEM((2, M, D), u32), pltpu.VMEM((2, C, D), u32), pltpu.VMEM((2, C, D), u32),
            pltpu.SemaphoreType.DMA((3, 2)),
            pltpu.VMEM((M, 3 * M), bf16), pltpu.VMEM((M, M), bf16), pltpu.VMEM((S, C), bf16),
            pltpu.SemaphoreType.DMA((3,))],
        compiler_params=pltpu.CompilerParams(dimension_semantics=("arbitrary",),
                                             vmem_limit_bytes=100 * 1024 * 1024),
    )(A_x[0].T, A_wqkv, A_wo, B_c_kv[0], B_w_q, B_w_uk, B_w_uv, B_w_o.transpose(0, 2, 1), gate_w.reshape(1, M))
    return out.T[None]
```
